```python
import os as _os
_os.environ.setdefault("JAX_PLATFORMS", "cpu")
import jax
import jax.numpy as jnp

def _softmax(x, axis=-1):
    return jax.nn.softmax(x, axis=axis)
def _gelu(x):
    return jax.nn.gelu(x, approximate=True)
def _silu(x):
    return jax.nn.silu(x)
def _sigmoid(x):
    return jax.nn.sigmoid(x)
def _layernorm(x, axis=-1, eps=1e-5):
    m = jnp.mean(x, axis=axis, keepdims=True)
    v = jnp.var(x, axis=axis, keepdims=True)
    return (x - m) / jnp.sqrt(v + eps)
def _scatter_add(tgt, idx, src, axis=0):
    return tgt.at[idx].add(src)
def _segment_sum(src, seg, n):
    return jax.ops.segment_sum(src, seg, n)
class _Rng:
    def __init__(self, key):
        self._k = key
    def _next(self):
        self._k, sub = jax.random.split(self._k)
        return sub
    def normal(self, shape):
        return jax.random.normal(self._next(), shape, dtype=jnp.bfloat16)
    def randint(self, lo, hi, shape):
        return jax.random.randint(self._next(), shape, lo, hi, dtype=jnp.int32)
    def uniform(self, shape, lo=0.0, hi=1.0):
        return jax.random.uniform(self._next(), shape, jnp.bfloat16, lo, hi)
    def permutation(self, n):
        return jax.random.permutation(self._next(), n)


kernel_name = 'concat_heads__linear_attn_block__sliding_local_dilated__prompt'

def setup_inputs():
    _rng = _Rng(jax.random.key(int.from_bytes(__import__("os").urandom(4), "little")))
    _w = (lambda a: (lambda t: t.astype(jnp.bfloat16) if jnp.issubdtype(t.dtype, jnp.floating) else t)(jnp.asarray(a)))
    def _A_setup():
        B, S, D = 1, 2048, 576
        return {
            "x": _w((lambda *s: _rng.normal(s) * 0.05)(B, S, D)),
            "wqkv": _w((lambda *s: _rng.normal(s) * 1.6)(D, 3 * D)),
            "wo": _w((lambda *s: _rng.normal(s) * 0.4)(D, D)),
        }
    _A_in = _A_setup()

    def _B_setup():
        B, S, D = 1, 2048, 576
        return {
            "x": _w((lambda *s: _rng.normal(s) * 0.2)(B, S, D)),
            "wqkv": _w((lambda *s: _rng.normal(s) * 0.2)(D, 3 * D)),
            "wo": _w((lambda *s: _rng.normal(s) * 0.05)(D, D)),
        }
    _B_in = _B_setup()

    return {
        "A_x": _A_in["x"],
        "A_wqkv": _A_in["wqkv"],
        "A_wo": _A_in["wo"],
        "B_x": _B_in["x"],
        "B_wqkv": _B_in["wqkv"],
        "B_wo": _B_in["wo"],
    }

def reference(A_x, A_wqkv, A_wo, B_x, B_wqkv, B_wo):
    def _A_ref(x, wqkv, wo):
        B, S, D = x.shape
        H = 32; Dh = D // H
        qkv = (lambda x, *d: x.transpose(*d))((x @ wqkv).reshape(B, S, 3, H, Dh), 2, 0, 3, 1, 4)
        q, k, v = qkv[0], qkv[1], qkv[2]
        phi = lambda t: jnp.where(t > 0, t + 1, jnp.exp(t)) + 1e-6
        pq, pk = phi(q), phi(k)
        kv = jnp.einsum("bhsd,bhse->bhde", pk, v)
        z = jnp.einsum("bhsd->bhd", pk)
        num = jnp.einsum("bhqd,bhde->bhqe", pq, kv)
        den = jnp.einsum("bhqd,bhd->bhq", pq, z)[..., None] + 1e-6
        o = num / den
        return (lambda x, *d: x.transpose(*d))(o, 0, 2, 1, 3).reshape(B, S, D) @ wo

    def _B_ref(x, wqkv, wo):
        B, S, D = x.shape
        H = 32; Dh = D // H
        W, dil = 8, 2
        qkv = (lambda x, *d: x.transpose(*d))((x @ wqkv).reshape(B, S, 3, H, Dh), 2, 0, 3, 1, 4)
        q, k, v = qkv[0], qkv[1], qkv[2]
        scale = Dh ** -0.5
        pos = jnp.arange(S)
        off = jnp.arange(W) * dil
        idx = pos[:, None] - off[None, :]
        mask = idx >= 0
        idx_c = jnp.where(mask, idx, 0).reshape(-1)
        kg = k[:, :, idx_c, :].reshape(B, H, S, W, Dh)
        vg = v[:, :, idx_c, :].reshape(B, H, S, W, Dh)
        logits = jnp.einsum("bhsd,bhswd->bhsw", q, kg) * scale
        logits = jnp.where(mask[None, None, :, :], logits, -1e9)
        attn = _softmax(logits, axis=-1)
        o = jnp.einsum("bhsw,bhswd->bhsd", attn, vg)
        return (lambda x, *d: x.transpose(*d))(o, 0, 2, 1, 3).reshape(B, S, D) @ wo

    a = _A_ref(A_x, A_wqkv, A_wo)
    b = _B_ref(B_x, B_wqkv, B_wo)
    return jnp.concatenate([a, b], axis=-1)
```

```python
import functools
import jax
import jax.numpy as jnp
from jax import lax
from jax.experimental import pallas as pl
from jax.experimental.pallas import tpu as pltpu

S = 2048
D = 576
H = 32
DH = 18
NT = 16
PITCH = 68
BF = jnp.bfloat16
F32 = jnp.float32
I32 = jnp.int32
NT_DIMS = (((1,), (1,)), ((), ()))
BAND = ((0, 144), (112, 272), (240, 400), (368, 528), (496, 576))
SCALE = float(DH) ** -0.5


def _phi(t):
    return jnp.where(t > 0, t + 1.0, jnp.exp(t)) + 1e-6


def _words(x):
    return pltpu.bitcast(x, I32)


def _unwords(x):
    return pltpu.bitcast(x, BF)


def _addall(xs):
    return functools.reduce(lambda a, b: a + b, xs)


def _kernel(xa_h, wa_h, woa_h, xb_h, wb_h, wob_h, out_h,
            xa_v, wa_v, woa_v, xb_v, wb_v, wob_v,
            wta, wtb, wotb, xs, kv, pkt, pw, zacc, zb, mt, qs, os0, os1, ob0, ob1, st, outv,
            sem_in, sem_out):
    XC = 512
    cp_wak = pltpu.make_async_copy(wa_h.at[:, pl.ds(512, 640)], wa_v.at[:, pl.ds(512, 640)], sem_in.at[0])
    cp_xa = [pltpu.make_async_copy(xa_h.at[:, pl.ds(XC * i, XC)], xa_v.at[:, pl.ds(XC * i, XC)], sem_in.at[1 + i])
             for i in range(S // XC)]
    cp_wb = pltpu.make_async_copy(wb_h, wb_v, sem_in.at[5])
    cp_xb = pltpu.make_async_copy(xb_h, xb_v, sem_in.at[6])
    cp_wob = pltpu.make_async_copy(wob_h, wob_v, sem_in.at[7])
    cp_waq = pltpu.make_async_copy(wa_h.at[:, pl.ds(0, 512)], wa_v.at[:, pl.ds(0, 512)], sem_in.at[8])
    cp_wav = pltpu.make_async_copy(wa_h.at[:, pl.ds(1152, 576)], wa_v.at[:, pl.ds(1152, 576)], sem_in.at[9])
    cp_woa = pltpu.make_async_copy(woa_h, woa_v, sem_in.at[10])
    cp_wak.start()
    for c in cp_xa:
        c.start()
    cp_wb.start()
    cp_xb.start()
    cp_wob.start()
    cp_waq.start()
    cp_wav.start()
    cp_woa.start()

    lane = lax.broadcasted_iota(I32, (8, 128), 1)

    cp_wak.wait()
    for c in range(4, 9):
        wta[pl.ds(64 * c, 64), :] = _words(wa_v[:, pl.ds(128 * c, 128)].T)
    zacc[...] = jnp.zeros((D, 128), F32)
    ob0[pl.ds(0, 64), :] = jnp.zeros((64, 128), F32)
    ob1[pl.ds(0, 64), :] = jnp.zeros((64, 128), F32)

    def p1(i, c):
        col = pl.ds(pl.multiple_of(i * XC, XC), XC)
        pltpu.make_async_copy(xa_h.at[:, col], xa_v.at[:, col], sem_in.at[1 + i]).wait()
        k = jnp.dot(_unwords(wta[pl.ds(D // 2, D // 2), :]), xa_v[:, col], preferred_element_type=F32)
        pk = _phi(k)
        pkt[:, col] = _words(pk.astype(BF))
        zacc[...] += _addall([pk[:, 128 * j:128 * j + 128] for j in range(XC // 128)])
        return c

    lax.fori_loop(0, S // XC, p1, 0)

    cp_wb.wait()
    cp_xb.wait()
    cp_wob.wait()
    cp_waq.wait()
    p = lax.dot_general(_unwords(pkt[...]), xa_v[...], NT_DIMS, preferred_element_type=F32)
    pw[...] = _words(p.astype(BF))
    zb[...] = jnp.broadcast_to(jnp.sum(zacc[...], axis=1, keepdims=True), (D, 128))
    for i in range(NT):
        wd = _words(xb_v[:, pl.ds(128 * i, 128)].T)
        for c in range(5):
            w = 128 if c < 4 else 64
            for r in range(8):
                start = 8 * (r % 2) * PITCH + 4 * i + r // 2
                xs[c, pl.ds(start, 8, stride=PITCH), pl.ds(0, w)] = wd[8 * r:8 * r + 8, 128 * c:128 * c + w]
    for c in range(14):
        w = 128 if c < 13 else 64
        wtb[pl.ds(64 * c, w // 2), :] = _words(wb_v[:, pl.ds(128 * c, w)].T)
    for c in range(5):
        w = 128 if c < 4 else 64
        wotb[pl.ds(64 * c, w // 2), :] = _words(wob_v[:, pl.ds(128 * c, w)].T)
    for c in range(4):
        wta[pl.ds(64 * c, 64), :] = _words(wa_v[:, pl.ds(128 * c, 128)].T)

    cp_wav.wait()
    cp_woa.wait()
    m_parts = []
    for jj in range(5):
        r0, r1 = BAND[jj]
        w = 128 if jj < 4 else 64
        g = jnp.dot(_unwords(pw[pl.ds(r0 // 2, (r1 - r0) // 2), :]), wa_v[:, pl.ds(2 * D + 128 * jj, w)],
                    preferred_element_type=F32)
        rr = lax.broadcasted_iota(I32, g.shape, 0) + r0
        cc = lax.broadcasted_iota(I32, g.shape, 1) + 128 * jj
        hr = lax.shift_right_logical(rr * 3641, 16)
        hc = lax.shift_right_logical(cc * 3641, 16)
        gb = jnp.where(hr == hc, g, 0.0).astype(BF)
        m_parts.append(jnp.dot(gb, woa_v[pl.ds(128 * jj, w), :], preferred_element_type=F32))
    cuts = sorted(set([b for r in BAND for b in r]))
    rows = []
    for a, b in zip(cuts[:-1], cuts[1:]):
        rows.append(_addall([m_parts[jj][a - BAND[jj][0]:b - BAND[jj][0], :] for jj in range(5)
                             if BAND[jj][0] <= a and b <= BAND[jj][1]]))
    mt[...] = _words(jnp.concatenate(rows, axis=0).astype(BF).T)

    def load_xs(u):
        rws = pl.ds(u * PITCH, 64)
        parts = [xs[c, rws, :] for c in range(4)] + [xs[4, rws, pl.ds(0, 64)]]
        return _unwords(jnp.concatenate(parts, axis=1))

    def p2(wrap, i, c):
        u = 2 * i
        xu = jnp.concatenate([load_xs(u), load_xs(u + 1)], axis=0)
        r = lax.dot_general(_unwords(wtb[pl.ds(D // 2, D), :]), xu, NT_DIMS, preferred_element_type=F32)
        for t in range(2):
            rt = r[:, 128 * t:128 * t + 128]
            kv[u + t + 8] = rt
            if wrap:
                kv[u + t - 8] = pltpu.roll(rt, 2, 1)
        return c

    lax.fori_loop(0, 4, functools.partial(p2, False), 0)
    lax.fori_loop(4, 8, functools.partial(p2, True), 0)

    def qproj_b(u):
        qs[...] = lax.dot_general(_unwords(wtb[pl.ds(0, D // 2), :]), load_xs(u), NT_DIMS,
                                  preferred_element_type=F32)

    def attn(u, os_):
        for g in range(4):
            q = [qs[pl.ds(d + DH * 8 * g, 8, stride=DH), :] for d in range(DH)]
            ls = []
            for w in range(8):
                l = _addall([q[d] * kv[u - w + 8, pl.ds(d + DH * 8 * g, 8, stride=DH), :] for d in range(DH)]) * SCALE
                if w > 0:
                    l = jnp.where(lane >= jnp.where(u < w, 2, 0), l, -1e9)
                ls.append(l)
            m = functools.reduce(jnp.maximum, ls)
            es = [jnp.exp(l - m) for l in ls]
            r = 1.0 / _addall(es)
            at = [e * r for e in es]
            for d in range(DH):
                os_[pl.ds(d + DH * 8 * g, 8, stride=DH), :] = _addall(
                    [at[w] * kv[u - w + 8, pl.ds(D + d + DH * 8 * g, 8, stride=DH), :] for w in range(8)])

    def oproj_b(os_, ob):
        ob[pl.ds(64, D), :] = jnp.dot(_unwords(wotb[...]), os_[...].astype(BF), preferred_element_type=F32)

    def otr_b(u, ob):
        wd = _words(ob[...].astype(BF).T)
        for cc in range(5):
            st[cc, pl.ds(u * PITCH, 64), :] = wd[:, 128 * cc:128 * cc + 128]

    qproj_b(0)
    attn(0, os0)
    qproj_b(1)
    attn(1, os1)
    oproj_b(os0, ob0)

    def p3(i, c):
        u = 2 * i
        qproj_b(u)
        attn(u, os0)
        oproj_b(os1, ob1)
        otr_b(u - 2, ob0)
        qproj_b(u + 1)
        attn(u + 1, os1)
        oproj_b(os0, ob0)
        otr_b(u - 1, ob1)
        return c

    lax.fori_loop(1, NT // 2, p3, 0)
    oproj_b(os1, ob1)
    otr_b(NT - 2, ob0)
    otr_b(NT - 1, ob1)

    def qphi(t, os_):
        col = pl.ds(pl.multiple_of(t * 128, 128), 128)
        qs[...] = jnp.dot(_unwords(wta[pl.ds(0, D // 2), :]), xa_v[:, col], preferred_element_type=F32)
        for g in range(4):
            pq = [_phi(qs[pl.ds(d + DH * 8 * g, 8, stride=DH), :]) for d in range(DH)]
            den = _addall([pq[d] * zb[pl.ds(d + DH * 8 * g, 8, stride=DH), :] for d in range(DH)])
            r = 1.0 / (den + 1e-6)
            for d in range(DH):
                os_[pl.ds(d + DH * 8 * g, 8, stride=DH), :] = pq[d] * r

    def oproj_a(os_, ob):
        ob[pl.ds(0, D), :] = jnp.dot(_unwords(mt[...]), os_[...].astype(BF), preferred_element_type=F32)

    def emit(t, ob):
        oa = ob[pl.ds(0, D), :].astype(BF).T
        rws = pl.ds(pl.multiple_of(t * 128, 128), 128)
        outv[rws, pl.ds(0, 512)] = oa[:, 0:512]
        bparts = []
        for cc in range(5):
            wl = [st[cc, pl.ds(8 * half * PITCH + 4 * t + jj, 8, stride=PITCH), :]
                  for jj in range(4) for half in range(2)]
            bparts.append(_unwords(jnp.concatenate(wl, axis=0)))
        a_tail = jnp.concatenate([oa[:, 512:576], jnp.zeros((128, 64), BF)], axis=1)
        outv[rws, pl.ds(512, 128)] = a_tail + bparts[0]
        for cc in range(1, 5):
            outv[rws, pl.ds(512 + 128 * cc, 128)] = bparts[cc]
        pltpu.make_async_copy(outv.at[rws, :], out_h.at[rws, :], sem_out.at[0]).start()

    qphi(0, os0)
    qphi(1, os1)
    oproj_a(os0, ob0)

    def p4(i, c):
        t = 2 * i
        qphi(t, os0)
        oproj_a(os1, ob1)
        emit(t - 2, ob0)
        qphi(t + 1, os1)
        oproj_a(os0, ob0)
        emit(t - 1, ob1)
        return c

    lax.fori_loop(1, NT // 2, p4, 0)
    oproj_a(os1, ob1)
    emit(NT - 2, ob0)
    emit(NT - 1, ob1)
    pltpu.make_async_copy(outv, out_h, sem_out.at[0]).wait()


def make():
    any_spec = pl.BlockSpec(memory_space=pl.ANY)
    return pl.pallas_call(
        _kernel,
        out_shape=jax.ShapeDtypeStruct((S, 2 * D), BF),
        in_specs=[any_spec] * 6,
        out_specs=any_spec,
        scratch_shapes=[
            pltpu.VMEM((D, S), BF), pltpu.VMEM((D, 3 * D), BF), pltpu.VMEM((D, D), BF),
            pltpu.VMEM((D, S), BF), pltpu.VMEM((D, 3 * D), BF), pltpu.VMEM((D, D), BF),
            pltpu.VMEM((D, D), I32),
            pltpu.VMEM((3 * D // 2, D), I32),
            pltpu.VMEM((D // 2, D), I32),
            pltpu.VMEM((5, NT * PITCH, 128), I32),
            pltpu.VMEM((24, 2 * D, 128), F32),
            pltpu.VMEM((D // 2, S), I32),
            pltpu.VMEM((D // 2, D), I32),
            pltpu.VMEM((D, 128), F32),
            pltpu.VMEM((D, 128), F32),
            pltpu.VMEM((D // 2, D), I32),
            pltpu.VMEM((D, 128), F32),
            pltpu.VMEM((D, 128), F32),
            pltpu.VMEM((D, 128), F32),
            pltpu.VMEM((D + 64, 128), F32),
            pltpu.VMEM((D + 64, 128), F32),
            pltpu.VMEM((5, NT * PITCH, 128), I32),
            pltpu.VMEM((S, 2 * D), BF),
            pltpu.SemaphoreType.DMA((11,)),
            pltpu.SemaphoreType.DMA((1,)),
        ],
        compiler_params=pltpu.CompilerParams(vmem_limit_bytes=100 * 1024 * 1024),
        name="fused_attn",
    )


@jax.jit
def pallas_concat_heads__linear_attn_block__sliding_local_dilated__prompt_kernel(A_x, A_wqkv, A_wo, B_x, B_wqkv, B_wo):
    out = make()(A_x[0].T, A_wqkv, A_wo, B_x[0].T, B_wqkv, B_wo)
    return out.reshape(1, S, 2 * D)
```

```python
import functools
import jax
import jax.numpy as jnp
from jax import lax
from jax.experimental import pallas as pl
from jax.experimental.pallas import tpu as pltpu

S = 2048
D = 576
H = 32
DH = 18
NT = 16
RPAD = 600
PITCH = 68
BF = jnp.bfloat16
F32 = jnp.float32
I32 = jnp.int32
NT_DIMS = (((1,), (1,)), ((), ()))
BAND = ((0, 144), (112, 272), (240, 400), (368, 528), (496, 576))
SCALE = float(DH) ** -0.5
LOG2E = 1.4426950408889634


def _phi(t):
    return jnp.where(t > 0, t + 1.0, jnp.exp(t)) + 1e-6


def _words(x):
    return pltpu.bitcast(x, I32)


def _unwords(x):
    return pltpu.bitcast(x, BF)


def _addall(xs):
    return functools.reduce(lambda a, b: a + b, xs)


def _maxall(xs):
    return functools.reduce(jnp.maximum, xs)


def _after(tok, xs):
    never = jnp.abs(tok) < -1.0
    return [jnp.where(never, 0.0, x) for x in xs]


def _kernel(xa_h, wa_h, woa_h, xb_h, wb_h, wob_h, out_h,
            xa_v, wa_v, woa_v, xb_v, wb_v, wob_v,
            wta, wtb, wotb, xs, kv, pkt, pw, zacc, zb, mt, qs, os0, os1, ob0, ob1, st, outv,
            sem_in, sem_out):
    XC = 512
    cp_wak = pltpu.make_async_copy(wa_h.at[:, pl.ds(512, 640)], wa_v.at[:, pl.ds(512, 640)], sem_in.at[0])
    cp_xa = [pltpu.make_async_copy(xa_h.at[:, pl.ds(XC * i, XC)], xa_v.at[:, pl.ds(XC * i, XC)], sem_in.at[1 + i])
             for i in range(S // XC)]
    cp_wb = pltpu.make_async_copy(wb_h.at[:, pl.ds(512, 1216)], wb_v.at[:, pl.ds(512, 1216)], sem_in.at[5])
    cp_wbq = pltpu.make_async_copy(wb_h.at[:, pl.ds(0, 512)], wb_v.at[:, pl.ds(0, 512)], sem_in.at[11])
    cp_xb = pltpu.make_async_copy(xb_h, xb_v, sem_in.at[6])
    cp_wob = pltpu.make_async_copy(wob_h, wob_v, sem_in.at[7])
    cp_waq = pltpu.make_async_copy(wa_h.at[:, pl.ds(0, 512)], wa_v.at[:, pl.ds(0, 512)], sem_in.at[8])
    cp_wav = pltpu.make_async_copy(wa_h.at[:, pl.ds(1152, 576)], wa_v.at[:, pl.ds(1152, 576)], sem_in.at[9])
    cp_woa = pltpu.make_async_copy(woa_h, woa_v, sem_in.at[10])
    cp_wak.start()
    cp_xa[0].start()

    lane = lax.broadcasted_iota(I32, (8, 128), 1)

    cp_wak.wait()
    for c in cp_xa[1:]:
        c.start()
    cp_wb.start()
    cp_xb.start()
    cp_wob.start()
    cp_waq.start()
    cp_wav.start()
    cp_woa.start()
    cp_wbq.start()
    for c in range(4, 9):
        wta[pl.ds(64 * c, 64), :] = _words(wa_v[:, pl.ds(128 * c, 128)].T)
    zacc[...] = jnp.zeros((D, 128), F32)
    ob0[pl.ds(0, 64), :] = jnp.zeros((64, 128), F32)
    ob1[...] = jnp.zeros((D + 64, 128), F32)

    def p1(i, c):
        col = pl.ds(pl.multiple_of(i * XC, XC), XC)
        pltpu.make_async_copy(xa_h.at[:, col], xa_v.at[:, col], sem_in.at[1 + i]).wait()
        k = jnp.dot(_unwords(wta[pl.ds(D // 2, D // 2), :]), xa_v[:, col], preferred_element_type=F32)
        pk = _phi(k)
        pkt[:, col] = _words(pk.astype(BF))
        zacc[...] += _addall([pk[:, 128 * j:128 * j + 128] for j in range(XC // 128)])
        return c

    lax.fori_loop(0, S // XC, p1, 0)

    cp_wb.wait()
    cp_xb.wait()
    p = lax.dot_general(_unwords(pkt[...]), xa_v[...], NT_DIMS, preferred_element_type=F32)
    pw[...] = _words(p.astype(BF))
    zb[pl.ds(0, D), :] = jnp.broadcast_to(jnp.sum(zacc[...], axis=1, keepdims=True), (D, 128))
    for i in range(NT):
        wd = _words(xb_v[:, pl.ds(128 * i, 128)].T)
        for c in range(5):
            w = 128 if c < 4 else 64
            for r in range(8):
                start = 8 * (r % 2) * PITCH + 4 * i + r // 2
                xs[c, pl.ds(start, 8, stride=PITCH), pl.ds(0, w)] = wd[8 * r:8 * r + 8, 128 * c:128 * c + w]
    for c in range(4, 14):
        w = 128 if c < 13 else 64
        wtb[pl.ds(64 * c, w // 2), :] = _words(wb_v[:, pl.ds(128 * c, w)].T)

    cp_wob.wait()
    cp_waq.wait()
    cp_wav.wait()
    cp_woa.wait()
    cp_wbq.wait()
    for c in range(4):
        wtb[pl.ds(64 * c, 64), :] = _words(wb_v[:, pl.ds(128 * c, 128)].T)
    for c in range(5):
        w = 128 if c < 4 else 64
        wotb[pl.ds(64 * c, w // 2), :] = _words(wob_v[:, pl.ds(128 * c, w)].T)
    for c in range(4):
        wta[pl.ds(64 * c, 64), :] = _words(wa_v[:, pl.ds(128 * c, 128)].T)
    g_parts = []
    for jj in range(5):
        r0, r1 = BAND[jj]
        w = 128 if jj < 4 else 64
        g = jnp.dot(_unwords(pw[pl.ds(r0 // 2, (r1 - r0) // 2), :]), wa_v[:, pl.ds(2 * D + 128 * jj, w)],
                    preferred_element_type=F32)
        rr = lax.broadcasted_iota(I32, g.shape, 0) + r0
        cc = lax.broadcasted_iota(I32, g.shape, 1) + 128 * jj
        hr = lax.shift_right_logical(rr * 3641, 16)
        hc = lax.shift_right_logical(cc * 3641, 16)
        gb = jnp.where(hr == hc, g, 0.0).astype(BF)
        g_parts.append(gb)
    def load_xs(u):
        rws = pl.ds(u * PITCH, 64)
        parts = [xs[c, rws, :] for c in range(4)] + [xs[4, rws, pl.ds(0, 64)]]
        return _unwords(jnp.concatenate(parts, axis=1))

    def p2(wrap, i, c):
        for half in range(2):
            u = 4 * i + 2 * half
            xu = jnp.concatenate([load_xs(u), load_xs(u + 1)], axis=0)
            r = lax.dot_general(_unwords(wtb[pl.ds(D // 2, D), :]), xu, NT_DIMS, preferred_element_type=F32)
            for t in range(2):
                rt = r[:, 128 * t:128 * t + 128]
                kv[u + t + 8, pl.ds(0, 2 * D), :] = rt
                if wrap:
                    kv[u + t - 8, pl.ds(0, 2 * D), :] = pltpu.roll(rt, 2, 1)
        return c

    m_parts = [jnp.dot(g_parts[jj], woa_v[pl.ds(128 * jj, 128 if jj < 4 else 64), :], preferred_element_type=F32)
               for jj in range(5)]
    cuts = sorted(set([b for r in BAND for b in r]))
    rows = []
    for a, b in zip(cuts[:-1], cuts[1:]):
        rows.append(_addall([m_parts[jj][a - BAND[jj][0]:b - BAND[jj][0], :] for jj in range(5)
                             if BAND[jj][0] <= a and b <= BAND[jj][1]]))
    mt[...] = _words(jnp.concatenate(rows, axis=0).astype(BF).T)

    for i in range(4):
        p2(i >= 2, i, 0)

    KL, KV, NM, NO = 4, 4, 3, 3
    MR = D // NM

    def qproj_b(u):
        xu = load_xs(u)
        for i in range(NM):
            qs[pl.ds(i * MR, MR), :] = lax.dot_general(_unwords(wtb[pl.ds(i * MR // 2, MR // 2), :]), xu, NT_DIMS,
                                                       preferred_element_type=F32)

    def attn(u, os_):
        last = None
        dk = [round(DH * i / KL) for i in range(KL + 1)]
        dv = [round(DH * i / KV) for i in range(KV + 1)]
        for g in range(4):
            q = [qs[pl.ds(d + DH * 8 * g, 8, stride=DH), :] for d in range(DH)]
            accs = [None] * 8
            for d0, d1 in zip(dk[:-1], dk[1:]):
                tok = last if d0 == 0 else _maxall(accs)
                qq = q[d0:d1]
                if tok is not None:
                    qq = _after(tok, qq)
                for w in range(8):
                    part = _addall([qq[d - d0] * kv[u - w + 8, pl.ds(d + DH * 8 * g, 8, stride=DH), :]
                                    for d in range(d0, d1)])
                    accs[w] = part if accs[w] is None else accs[w] + part
            ls = [accs[0]] + [jnp.where(lane >= jnp.where(u < w, 2, 0), accs[w], -1e9 / SCALE) for w in range(1, 8)]
            m = _maxall(ls)
            es = [jnp.exp2((l - m) * (SCALE * LOG2E)) for l in ls]
            r = 1.0 / _addall(es)
            at = [e * r for e in es]
            for d0, d1 in zip(dv[:-1], dv[1:]):
                outs = []
                for d in range(d0, d1):
                    o = _addall([at[w] * kv[u - w + 8, pl.ds(D + d + DH * 8 * g, 8, stride=DH), :] for w in range(8)])
                    os_[pl.ds(d + DH * 8 * g, 8, stride=DH), :] = o
                    outs.append(o)
                last = _maxall(outs)
                if d1 < DH:
                    at = _after(last, at)

    def oproj_b(os_, ob):
        rhs = os_[pl.ds(0, D), :].astype(BF)
        MR = D // NO
        for i in range(NO):
            ob[pl.ds(64 + i * MR, MR), :] = jnp.dot(_unwords(wotb[pl.ds(i * MR // 2, MR // 2), :]), rhs,
                                                    preferred_element_type=F32)

    def otr_b(u, ob):
        wd = _words(ob[...].astype(BF).T)
        for cc in range(5):
            st[cc, pl.ds(u * PITCH, 64), :] = wd[:, 128 * cc:128 * cc + 128]

    qproj_b(0)
    attn(0, os0)
    qproj_b(1)
    attn(1, os1)
    oproj_b(os0, ob0)

    def p3(i, c):
        u = 2 * i
        ops = {'q': lambda k: qproj_b(u + k), 'a': lambda k: attn(u + k, (os0, os1)[k]),
               'o': lambda k: oproj_b((os1, os0)[k], (ob1, ob0)[k]), 't': lambda k: otr_b(u + k - 2, (ob0, ob1)[k])}
        for k in range(2):
            for ch in 'qaot':
                ops[ch](k)
        return c

    lax.fori_loop(1, NT // 2, p3, 0)
    oproj_b(os1, ob1)
    otr_b(NT - 2, ob0)
    otr_b(NT - 1, ob1)

    def qphi(t, os_):
        col = pl.ds(pl.multiple_of(t * 128, 128), 128)
        xt = xa_v[:, col]
        qs[pl.ds(0, D), :] = jnp.dot(_unwords(wta[pl.ds(0, D // 2), :]), xt, preferred_element_type=F32)
        for g in range(4):
            pq = [_phi(qs[pl.ds(d + DH * 8 * g, 8, stride=DH), :]) for d in range(DH)]
            den = _addall([pq[d] * zb[pl.ds(d + DH * 8 * g, 8, stride=DH), :] for d in range(DH)])
            r = 1.0 / (den + 1e-6)
            for d in range(DH):
                os_[pl.ds(d + DH * 8 * g, 8, stride=DH), :] = pq[d] * r

    def oproj_a(os_, ob):
        rhs = os_[pl.ds(0, D), :].astype(BF)
        ob[pl.ds(0, D), :] = jnp.dot(_unwords(mt[...]), rhs, preferred_element_type=F32)

    def emit(t, ob):
        oa = _words(ob[...].astype(BF).T)
        rws = pl.ds(pl.multiple_of(t * 128, 128), 128)
        outv[rws, pl.ds(0, 512)] = _unwords(oa[:, 0:512])
        for cc in range(5):
            wl = jnp.concatenate([st[cc, pl.ds(8 * half * PITCH + 4 * t + jj, 8, stride=PITCH), :]
                                  for jj in range(4) for half in range(2)], axis=0)
            if cc == 0:
                wl = wl | oa[:, 512:640]
            outv[rws, pl.ds(512 + 128 * cc, 128)] = _unwords(wl)

    def send(t):
        rws = pl.ds(pl.multiple_of(t * 128, 128), 128)
        pltpu.make_async_copy(outv.at[rws, :], out_h.at[rws, :], sem_out.at[0]).start()

    ob0[pl.ds(D, 64), :] = jnp.zeros((64, 128), F32)
    ob1[pl.ds(D, 64), :] = jnp.zeros((64, 128), F32)
    qphi(0, os0)
    qphi(1, os1)
    oproj_a(os0, ob0)

    def p4(i, c):
        t = 2 * i
        qphi(t, os0)
        oproj_a(os1, ob1)
        emit(t - 2, ob0)
        qphi(t + 1, os1)
        oproj_a(os0, ob0)
        emit(t - 1, ob1)
        send(t - 1)
        send(t - 2)
        return c

    lax.fori_loop(1, NT // 2, p4, 0)
    emit(NT - 2, ob0)
    send(NT - 2)
    oproj_a(os1, ob1)
    emit(NT - 1, ob1)
    send(NT - 1)
    pltpu.make_async_copy(outv, out_h, sem_out.at[0]).wait()


def make():
    any_spec = pl.BlockSpec(memory_space=pl.ANY)
    return pl.pallas_call(
        _kernel,
        out_shape=jax.ShapeDtypeStruct((S, 2 * D), BF),
        in_specs=[any_spec] * 6,
        out_specs=any_spec,
        scratch_shapes=[
            pltpu.VMEM((D, S), BF), pltpu.VMEM((D, 3 * D), BF), pltpu.VMEM((D, D), BF),
            pltpu.VMEM((D, S), BF), pltpu.VMEM((D, 3 * D), BF), pltpu.VMEM((D, D), BF),
            pltpu.VMEM((D, D), I32),
            pltpu.VMEM((3 * D // 2, D), I32),
            pltpu.VMEM((D // 2, D), I32),
            pltpu.VMEM((5, (NT + 1) * PITCH, 128), I32),
            pltpu.VMEM((24, D + RPAD, 128), F32),
            pltpu.VMEM((D // 2, S), I32),
            pltpu.VMEM((D // 2, D), I32),
            pltpu.VMEM((D, 128), F32),
            pltpu.VMEM((RPAD, 128), F32),
            pltpu.VMEM((D // 2, D), I32),
            pltpu.VMEM((RPAD, 128), F32),
            pltpu.VMEM((RPAD, 128), F32),
            pltpu.VMEM((RPAD, 128), F32),
            pltpu.VMEM((D + 64, 128), F32),
            pltpu.VMEM((D + 64, 128), F32),
            pltpu.VMEM((5, (NT + 1) * PITCH, 128), I32),
            pltpu.VMEM((S, 2 * D), BF),
            pltpu.SemaphoreType.DMA((12,)),
            pltpu.SemaphoreType.DMA((1,)),
        ],
        compiler_params=pltpu.CompilerParams(vmem_limit_bytes=100 * 1024 * 1024),
        name="fused_attn",
    )


@jax.jit
def pallas_concat_heads__linear_attn_block__sliding_local_dilated__prompt_kernel(A_x, A_wqkv, A_wo, B_x, B_wqkv, B_wo):
    out = make()(A_x[0].T, A_wqkv, A_wo, B_x[0].T, B_wqkv, B_wo)
    return out.reshape(1, S, 2 * D)
```

```python
import functools
import jax
import jax.numpy as jnp
from jax import lax
from jax.experimental import pallas as pl
from jax.experimental.pallas import tpu as pltpu

S = 2048
D = 576
H = 32
DH = 18
NT = 16
RPAD = 600
PITCH = 68
BF = jnp.bfloat16
F32 = jnp.float32
I32 = jnp.int32
NT_DIMS = (((1,), (1,)), ((), ()))
BAND = ((0, 144), (112, 272), (240, 400), (368, 528), (496, 576))
SCALE = float(DH) ** -0.5
LOG2E = 1.4426950408889634


def _phi(t):
    return jnp.where(t > 0, t + 1.0, jnp.exp(t)) + 1e-6


def _words(x):
    return pltpu.bitcast(x, I32)


def _unwords(x):
    return pltpu.bitcast(x, BF)


def _addall(xs):
    return functools.reduce(lambda a, b: a + b, xs)


def _maxall(xs):
    return functools.reduce(jnp.maximum, xs)


def _after(tok, xs):
    never = jnp.abs(tok) < -1.0
    return [jnp.where(never, 0.0, x) for x in xs]


def _kernel(xa_h, wa_h, woa_h, xb_h, wb_h, wob_h, out_h,
            xa_v, wa_v, woa_v, xb_v, wb_v, wob_v,
            wta, wtb, wotb, xs, kv, pkt, pw, zacc, zb, mt, qs, os0, os1, ob0, ob1, st, outv,
            sem_in, sem_out):
    XC = 512
    cp_wak = pltpu.make_async_copy(wa_h.at[:, pl.ds(512, 640)], wa_v.at[:, pl.ds(512, 640)], sem_in.at[0])
    cp_xa = [pltpu.make_async_copy(xa_h.at[:, pl.ds(XC * i, XC)], xa_v.at[:, pl.ds(XC * i, XC)], sem_in.at[1 + i])
             for i in range(S // XC)]
    cp_wb = pltpu.make_async_copy(wb_h.at[:, pl.ds(512, 1216)], wb_v.at[:, pl.ds(512, 1216)], sem_in.at[5])
    cp_wbq = pltpu.make_async_copy(wb_h.at[:, pl.ds(0, 512)], wb_v.at[:, pl.ds(0, 512)], sem_in.at[11])
    cp_xb = pltpu.make_async_copy(xb_h, xb_v, sem_in.at[6])
    cp_wob = pltpu.make_async_copy(wob_h, wob_v, sem_in.at[7])
    cp_waq = pltpu.make_async_copy(wa_h.at[:, pl.ds(0, 512)], wa_v.at[:, pl.ds(0, 512)], sem_in.at[8])
    cp_wav = pltpu.make_async_copy(wa_h.at[:, pl.ds(1152, 576)], wa_v.at[:, pl.ds(1152, 576)], sem_in.at[9])
    cp_woa = pltpu.make_async_copy(woa_h, woa_v, sem_in.at[10])
    cp_wak.start()
    cp_xa[0].start()

    lane = lax.broadcasted_iota(I32, (8, 128), 1)

    cp_wak.wait()
    for c in cp_xa[1:]:
        c.start()
    cp_wb.start()
    cp_xb.start()
    cp_wob.start()
    cp_waq.start()
    cp_wav.start()
    cp_woa.start()
    cp_wbq.start()
    for c in range(4, 9):
        wta[pl.ds(64 * c, 64), :] = _words(wa_v[:, pl.ds(128 * c, 128)].T)
    zacc[...] = jnp.zeros((D, 128), F32)
    ob0[pl.ds(0, 64), :] = jnp.zeros((64, 128), F32)
    ob1[...] = jnp.zeros((D + 64, 128), F32)

    def p1(i, c):
        col = pl.ds(pl.multiple_of(i * XC, XC), XC)
        pltpu.make_async_copy(xa_h.at[:, col], xa_v.at[:, col], sem_in.at[1 + i]).wait()
        k = jnp.dot(_unwords(wta[pl.ds(D // 2, D // 2), :]), xa_v[:, col], preferred_element_type=F32)
        pk = _phi(k)
        pkt[:, col] = _words(pk.astype(BF))
        zacc[...] += _addall([pk[:, 128 * j:128 * j + 128] for j in range(XC // 128)])
        return c

    lax.fori_loop(0, S // XC, p1, 0)

    cp_wb.wait()
    cp_xb.wait()
    p = lax.dot_general(_unwords(pkt[...]), xa_v[...], NT_DIMS, preferred_element_type=F32)
    pw[...] = _words(p.astype(BF))
    zb[pl.ds(0, D), :] = jnp.broadcast_to(jnp.sum(zacc[...], axis=1, keepdims=True), (D, 128))
    for i in range(NT):
        wd = _words(xb_v[:, pl.ds(128 * i, 128)].T)
        for c in range(5):
            w = 128 if c < 4 else 64
            for r in range(8):
                start = 8 * (r % 2) * PITCH + 4 * i + r // 2
                xs[c, pl.ds(start, 8, stride=PITCH), pl.ds(0, w)] = wd[8 * r:8 * r + 8, 128 * c:128 * c + w]
    for c in range(4, 14):
        w = 128 if c < 13 else 64
        wtb[pl.ds(64 * c, w // 2), :] = _words(wb_v[:, pl.ds(128 * c, w)].T)

    cp_wob.wait()
    cp_waq.wait()
    cp_wav.wait()
    cp_woa.wait()
    cp_wbq.wait()
    for c in range(4):
        wtb[pl.ds(64 * c, 64), :] = _words(wb_v[:, pl.ds(128 * c, 128)].T)
    for c in range(5):
        w = 128 if c < 4 else 64
        wotb[pl.ds(64 * c, w // 2), :] = _words(wob_v[:, pl.ds(128 * c, w)].T)
    for c in range(4):
        wta[pl.ds(64 * c, 64), :] = _words(wa_v[:, pl.ds(128 * c, 128)].T)
    g_parts = []
    for jj in range(5):
        r0, r1 = BAND[jj]
        w = 128 if jj < 4 else 64
        g = jnp.dot(_unwords(pw[pl.ds(r0 // 2, (r1 - r0) // 2), :]), wa_v[:, pl.ds(2 * D + 128 * jj, w)],
                    preferred_element_type=F32)
        rr = lax.broadcasted_iota(I32, g.shape, 0) + r0
        cc = lax.broadcasted_iota(I32, g.shape, 1) + 128 * jj
        hr = lax.shift_right_logical(rr * 3641, 16)
        hc = lax.shift_right_logical(cc * 3641, 16)
        gb = jnp.where(hr == hc, g, 0.0).astype(BF)
        g_parts.append(gb)
    def load_xs(u):
        rws = pl.ds(u * PITCH, 64)
        parts = [xs[c, rws, :] for c in range(4)] + [xs[4, rws, pl.ds(0, 64)]]
        return _unwords(jnp.concatenate(parts, axis=1))

    def p2(u):
        xu = jnp.concatenate([load_xs(u), load_xs(u + 1)], axis=0)
        r = lax.dot_general(_unwords(wtb[pl.ds(D // 2, D), :]), xu, NT_DIMS, preferred_element_type=F32)
        for t in range(2):
            rt = r[:, 128 * t:128 * t + 128]
            kv[u + t + 8, pl.ds(0, 2 * D), :] = rt
            if u + t > 8:
                kv[u + t - 8, pl.ds(0, 2 * D), :] = pltpu.roll(rt, 2, 1)

    m_parts = [jnp.dot(g_parts[jj], woa_v[pl.ds(128 * jj, 128 if jj < 4 else 64), :], preferred_element_type=F32)
               for jj in range(5)]
    cuts = sorted(set([b for r in BAND for b in r]))
    rows = []
    for a, b in zip(cuts[:-1], cuts[1:]):
        rows.append(_addall([m_parts[jj][a - BAND[jj][0]:b - BAND[jj][0], :] for jj in range(5)
                             if BAND[jj][0] <= a and b <= BAND[jj][1]]))
    mt[...] = _words(jnp.concatenate(rows, axis=0).astype(BF).T)

    for u in (8, 10, 12, 14, 0, 2):
        p2(u)

    KL, KV, NM, NO = 4, 4, 3, 3
    MR = D // NM

    def qproj_b(u):
        xu = load_xs(u)
        for i in range(NM):
            qs[pl.ds(i * MR, MR), :] = lax.dot_general(_unwords(wtb[pl.ds(i * MR // 2, MR // 2), :]), xu, NT_DIMS,
                                                       preferred_element_type=F32)

    def attn(u, os_):
        last = None
        dk = [round(DH * i / KL) for i in range(KL + 1)]
        dv = [round(DH * i / KV) for i in range(KV + 1)]
        for g in range(4):
            q = [qs[pl.ds(d + DH * 8 * g, 8, stride=DH), :] for d in range(DH)]
            accs = [None] * 8
            for d0, d1 in zip(dk[:-1], dk[1:]):
                tok = last if d0 == 0 else _maxall(accs)
                qq = q[d0:d1]
                if tok is not None:
                    qq = _after(tok, qq)
                for w in range(8):
                    part = _addall([qq[d - d0] * kv[u - w + 8, pl.ds(d + DH * 8 * g, 8, stride=DH), :]
                                    for d in range(d0, d1)])
                    accs[w] = part if accs[w] is None else accs[w] + part
            ls = [accs[0]] + [jnp.where(lane >= jnp.where(u < w, 2, 0), accs[w], -1e9 / SCALE) for w in range(1, 8)]
            m = _maxall(ls)
            es = [jnp.exp2((l - m) * (SCALE * LOG2E)) for l in ls]
            r = 1.0 / _addall(es)
            at = [e * r for e in es]
            for d0, d1 in zip(dv[:-1], dv[1:]):
                outs = []
                for d in range(d0, d1):
                    o = _addall([at[w] * kv[u - w + 8, pl.ds(D + d + DH * 8 * g, 8, stride=DH), :] for w in range(8)])
                    os_[pl.ds(d + DH * 8 * g, 8, stride=DH), :] = o
                    outs.append(o)
                last = _maxall(outs)
                if d1 < DH:
                    at = _after(last, at)

    def oproj_b(os_, ob):
        rhs = os_[pl.ds(0, D), :].astype(BF)
        MR = D // NO
        for i in range(NO):
            ob[pl.ds(64 + i * MR, MR), :] = jnp.dot(_unwords(wotb[pl.ds(i * MR // 2, MR // 2), :]), rhs,
                                                    preferred_element_type=F32)

    def otr_b(u, ob):
        wd = _words(ob[...].astype(BF).T)
        for cc in range(5):
            st[cc, pl.ds(u * PITCH, 64), :] = wd[:, 128 * cc:128 * cc + 128]

    qproj_b(0)
    attn(0, os0)
    p2(4)
    qproj_b(1)
    attn(1, os1)
    p2(6)
    oproj_b(os0, ob0)

    def p3(i, c):
        u = 2 * i
        ops = {'q': lambda k: qproj_b(u + k), 'a': lambda k: attn(u + k, (os0, os1)[k]),
               'o': lambda k: oproj_b((os1, os0)[k], (ob1, ob0)[k]), 't': lambda k: otr_b(u + k - 2, (ob0, ob1)[k])}
        for k in range(2):
            for ch in 'qaot':
                ops[ch](k)
        return c

    lax.fori_loop(1, NT // 2, p3, 0)
    oproj_b(os1, ob1)
    otr_b(NT - 2, ob0)
    otr_b(NT - 1, ob1)

    def qphi(t, os_):
        col = pl.ds(pl.multiple_of(t * 128, 128), 128)
        xt = xa_v[:, col]
        qs[pl.ds(0, D), :] = jnp.dot(_unwords(wta[pl.ds(0, D // 2), :]), xt, preferred_element_type=F32)
        for g in range(4):
            pq = [_phi(qs[pl.ds(d + DH * 8 * g, 8, stride=DH), :]) for d in range(DH)]
            den = _addall([pq[d] * zb[pl.ds(d + DH * 8 * g, 8, stride=DH), :] for d in range(DH)])
            r = 1.0 / (den + 1e-6)
            for d in range(DH):
                os_[pl.ds(d + DH * 8 * g, 8, stride=DH), :] = pq[d] * r

    def oproj_a(os_, ob):
        rhs = os_[pl.ds(0, D), :].astype(BF)
        ob[pl.ds(0, D), :] = jnp.dot(_unwords(mt[...]), rhs, preferred_element_type=F32)

    def emit(t, ob):
        oa = _words(ob[...].astype(BF).T)
        rws = pl.ds(pl.multiple_of(t * 128, 128), 128)
        outv[rws, pl.ds(0, 512)] = _unwords(oa[:, 0:512])
        for cc in range(5):
            wl = jnp.concatenate([st[cc, pl.ds(8 * half * PITCH + 4 * t + jj, 8, stride=PITCH), :]
                                  for jj in range(4) for half in range(2)], axis=0)
            if cc == 0:
                wl = wl | oa[:, 512:640]
            outv[rws, pl.ds(512 + 128 * cc, 128)] = _unwords(wl)

    def send(t):
        rws = pl.ds(pl.multiple_of(t * 128, 128), 128)
        pltpu.make_async_copy(outv.at[rws, :], out_h.at[rws, :], sem_out.at[0]).start()

    ob0[pl.ds(D, 64), :] = jnp.zeros((64, 128), F32)
    ob1[pl.ds(D, 64), :] = jnp.zeros((64, 128), F32)
    qphi(0, os0)
    qphi(1, os1)
    oproj_a(os0, ob0)

    def p4(i, c):
        t = 2 * i
        qphi(t, os0)
        oproj_a(os1, ob1)
        emit(t - 2, ob0)
        qphi(t + 1, os1)
        oproj_a(os0, ob0)
        emit(t - 1, ob1)
        send(t - 1)
        send(t - 2)
        return c

    lax.fori_loop(1, NT // 2, p4, 0)
    emit(NT - 2, ob0)
    send(NT - 2)
    oproj_a(os1, ob1)
    emit(NT - 1, ob1)
    send(NT - 1)
    pltpu.make_async_copy(outv, out_h, sem_out.at[0]).wait()


def make():
    any_spec = pl.BlockSpec(memory_space=pl.ANY)
    return pl.pallas_call(
        _kernel,
        out_shape=jax.ShapeDtypeStruct((S, 2 * D), BF),
        in_specs=[any_spec] * 6,
        out_specs=any_spec,
        scratch_shapes=[
            pltpu.VMEM((D, S), BF), pltpu.VMEM((D, 3 * D), BF), pltpu.VMEM((D, D), BF),
            pltpu.VMEM((D, S), BF), pltpu.VMEM((D, 3 * D), BF), pltpu.VMEM((D, D), BF),
            pltpu.VMEM((D, D), I32),
            pltpu.VMEM((3 * D // 2, D), I32),
            pltpu.VMEM((D // 2, D), I32),
            pltpu.VMEM((5, (NT + 1) * PITCH, 128), I32),
            pltpu.VMEM((24, D + RPAD, 128), F32),
            pltpu.VMEM((D // 2, S), I32),
            pltpu.VMEM((D // 2, D), I32),
            pltpu.VMEM((D, 128), F32),
            pltpu.VMEM((RPAD, 128), F32),
            pltpu.VMEM((D // 2, D), I32),
            pltpu.VMEM((RPAD, 128), F32),
            pltpu.VMEM((RPAD, 128), F32),
            pltpu.VMEM((RPAD, 128), F32),
            pltpu.VMEM((D + 64, 128), F32),
            pltpu.VMEM((D + 64, 128), F32),
            pltpu.VMEM((5, (NT + 1) * PITCH, 128), I32),
            pltpu.VMEM((S, 2 * D), BF),
            pltpu.SemaphoreType.DMA((12,)),
            pltpu.SemaphoreType.DMA((1,)),
        ],
        compiler_params=pltpu.CompilerParams(vmem_limit_bytes=100 * 1024 * 1024),
        name="fused_attn",
    )


@jax.jit
def pallas_concat_heads__linear_attn_block__sliding_local_dilated__prompt_kernel(A_x, A_wqkv, A_wo, B_x, B_wqkv, B_wo):
    out = make()(A_x[0].T, A_wqkv, A_wo, B_x[0].T, B_wqkv, B_wo)
    return out.reshape(1, S, 2 * D)
```

```python
import functools
import jax
import jax.numpy as jnp
from jax import lax
from jax.experimental import pallas as pl
from jax.experimental.pallas import tpu as pltpu

S = 2048
D = 576
H = 32
DH = 18
NT = 16
RPAD = 600
PITCH = 68
BF = jnp.bfloat16
F32 = jnp.float32
I32 = jnp.int32
NT_DIMS = (((1,), (1,)), ((), ()))
BAND = ((0, 144), (112, 272), (240, 400), (368, 528), (496, 576))
SCALE = float(DH) ** -0.5
LOG2E = 1.4426950408889634


def _phi(t):
    return jnp.where(t > 0, t + 1.0, jnp.exp(t)) + 1e-6


def _words(x):
    return pltpu.bitcast(x, I32)


def _unwords(x):
    return pltpu.bitcast(x, BF)


def _addall(xs):
    return functools.reduce(lambda a, b: a + b, xs)


def _maxall(xs):
    return functools.reduce(jnp.maximum, xs)


def _after(tok, xs):
    never = jnp.abs(tok) < -1.0
    return [jnp.where(never, 0.0, x) for x in xs]


def _kernel(xa_h, wa_h, woa_h, xb_h, wb_h, wob_h, out_h,
            xa_v, wa_v, woa_v, xb_v, wb_v, wob_v,
            wta, wtb, wotb, xs, kv, pkt, pw, zacc, zb, mt, qs, os0, os1, ob0, ob1, st, outv,
            sem_in, sem_out):
    XC = 512
    cp_wak = pltpu.make_async_copy(wa_h.at[:, pl.ds(512, 640)], wa_v.at[:, pl.ds(512, 640)], sem_in.at[0])
    cp_xa = [pltpu.make_async_copy(xa_h.at[:, pl.ds(XC * i, XC)], xa_v.at[:, pl.ds(XC * i, XC)], sem_in.at[1 + i])
             for i in range(S // XC)]
    cp_wb = pltpu.make_async_copy(wb_h.at[:, pl.ds(512, 1216)], wb_v.at[:, pl.ds(512, 1216)], sem_in.at[5])
    cp_wbq = pltpu.make_async_copy(wb_h.at[:, pl.ds(0, 512)], wb_v.at[:, pl.ds(0, 512)], sem_in.at[11])
    cp_xb = pltpu.make_async_copy(xb_h, xb_v, sem_in.at[6])
    cp_wob = pltpu.make_async_copy(wob_h, wob_v, sem_in.at[7])
    cp_waq = pltpu.make_async_copy(wa_h.at[:, pl.ds(0, 512)], wa_v.at[:, pl.ds(0, 512)], sem_in.at[8])
    cp_wav = pltpu.make_async_copy(wa_h.at[:, pl.ds(1152, 576)], wa_v.at[:, pl.ds(1152, 576)], sem_in.at[9])
    cp_woa = pltpu.make_async_copy(woa_h, woa_v, sem_in.at[10])
    cp_wak.start()
    cp_xa[0].start()

    lane = lax.broadcasted_iota(I32, (8, 128), 1)

    cp_wak.wait()
    for c in cp_xa[1:]:
        c.start()
    cp_wb.start()
    cp_xb.start()
    cp_wob.start()
    cp_waq.start()
    cp_wav.start()
    cp_woa.start()
    cp_wbq.start()
    for c in range(4, 9):
        wta[pl.ds(64 * c, 64), :] = _words(wa_v[:, pl.ds(128 * c, 128)].T)
    zacc[...] = jnp.zeros((D, 128), F32)
    ob0[pl.ds(0, 64), :] = jnp.zeros((64, 128), F32)
    ob1[...] = jnp.zeros((D + 64, 128), F32)

    def p1(i, c):
        col = pl.ds(pl.multiple_of(i * XC, XC), XC)
        pltpu.make_async_copy(xa_h.at[:, col], xa_v.at[:, col], sem_in.at[1 + i]).wait()
        k = jnp.dot(_unwords(wta[pl.ds(D // 2, D // 2), :]), xa_v[:, col], preferred_element_type=F32)
        pk = _phi(k)
        pkt[:, col] = _words(pk.astype(BF))
        zacc[...] += _addall([pk[:, 128 * j:128 * j + 128] for j in range(XC // 128)])
        return c

    lax.fori_loop(0, S // XC, p1, 0)

    cp_wb.wait()
    cp_xb.wait()
    p = lax.dot_general(_unwords(pkt[...]), xa_v[...], NT_DIMS, preferred_element_type=F32)
    pw[...] = _words(p.astype(BF))
    zb[pl.ds(0, D), :] = jnp.broadcast_to(jnp.sum(zacc[...], axis=1, keepdims=True), (D, 128))
    for i in range(NT):
        wd = _words(xb_v[:, pl.ds(128 * i, 128)].T)
        for c in range(5):
            w = 128 if c < 4 else 64
            for r in range(8):
                start = 8 * (r % 2) * PITCH + 4 * i + r // 2
                xs[c, pl.ds(start, 8, stride=PITCH), pl.ds(0, w)] = wd[8 * r:8 * r + 8, 128 * c:128 * c + w]
    for c in range(4, 14):
        w = 128 if c < 13 else 64
        wtb[pl.ds(64 * c, w // 2), :] = _words(wb_v[:, pl.ds(128 * c, w)].T)

    cp_wob.wait()
    cp_waq.wait()
    cp_wav.wait()
    cp_woa.wait()
    cp_wbq.wait()
    for c in range(4):
        wtb[pl.ds(64 * c, 64), :] = _words(wb_v[:, pl.ds(128 * c, 128)].T)
    for c in range(5):
        w = 128 if c < 4 else 64
        wotb[pl.ds(64 * c, w // 2), :] = _words(wob_v[:, pl.ds(128 * c, w)].T)
    for c in range(4):
        wta[pl.ds(64 * c, 64), :] = _words(wa_v[:, pl.ds(128 * c, 128)].T)
    g_parts = []
    for jj in range(5):
        r0, r1 = BAND[jj]
        w = 128 if jj < 4 else 64
        g = jnp.dot(_unwords(pw[pl.ds(r0 // 2, (r1 - r0) // 2), :]), wa_v[:, pl.ds(2 * D + 128 * jj, w)],
                    preferred_element_type=F32)
        rr = lax.broadcasted_iota(I32, g.shape, 0) + r0
        cc = lax.broadcasted_iota(I32, g.shape, 1) + 128 * jj
        hr = lax.shift_right_logical(rr * 3641, 16)
        hc = lax.shift_right_logical(cc * 3641, 16)
        gb = jnp.where(hr == hc, g, 0.0).astype(BF)
        g_parts.append(gb)
    def load_xs(u):
        rws = pl.ds(u * PITCH, 64)
        parts = [xs[c, rws, :] for c in range(4)] + [xs[4, rws, pl.ds(0, 64)]]
        return _unwords(jnp.concatenate(parts, axis=1))

    def p2(u):
        xu = jnp.concatenate([load_xs(u), load_xs(u + 1)], axis=0)
        r = lax.dot_general(_unwords(wtb[pl.ds(D // 2, D), :]), xu, NT_DIMS, preferred_element_type=F32)
        for t in range(2):
            rt = r[:, 128 * t:128 * t + 128]
            kv[u + t + 8, pl.ds(0, 2 * D), :] = rt
            if u + t > 8:
                kv[u + t - 8, pl.ds(0, 2 * D), :] = pltpu.roll(rt, 2, 1)

    m_parts = [jnp.dot(g_parts[jj], woa_v[pl.ds(128 * jj, 128 if jj < 4 else 64), :], preferred_element_type=F32)
               for jj in range(5)]
    cuts = sorted(set([b for r in BAND for b in r]))
    rows = []
    for a, b in zip(cuts[:-1], cuts[1:]):
        rows.append(_addall([m_parts[jj][a - BAND[jj][0]:b - BAND[jj][0], :] for jj in range(5)
                             if BAND[jj][0] <= a and b <= BAND[jj][1]]))
    mt[...] = _words(jnp.concatenate(rows, axis=0).astype(BF).T)

    for u in (8, 10, 12, 14, 0, 2):
        p2(u)

    KL, KV, NM, NO = 4, 4, 3, 3
    MR = D // NM

    def qproj_b(u):
        xu = load_xs(u)
        for i in range(NM):
            qs[pl.ds(i * MR, MR), :] = lax.dot_general(_unwords(wtb[pl.ds(i * MR // 2, MR // 2), :]), xu, NT_DIMS,
                                                       preferred_element_type=F32)

    def attn(u, os_):
        last = None
        dk = [round(DH * i / KL) for i in range(KL + 1)]
        dv = [round(DH * i / KV) for i in range(KV + 1)]
        for g in range(4):
            q = [qs[pl.ds(d + DH * 8 * g, 8, stride=DH), :] for d in range(DH)]
            accs = [None] * 8
            for d0, d1 in zip(dk[:-1], dk[1:]):
                tok = last if d0 == 0 else _maxall(accs)
                qq = q[d0:d1]
                if tok is not None:
                    qq = _after(tok, qq)
                for w in range(8):
                    part = _addall([qq[d - d0] * kv[u - w + 8, pl.ds(d + DH * 8 * g, 8, stride=DH), :]
                                    for d in range(d0, d1)])
                    accs[w] = part if accs[w] is None else accs[w] + part
            ls = [accs[0]] + [jnp.where(lane >= jnp.where(u < w, 2, 0), accs[w], -1e9 / SCALE) for w in range(1, 8)]
            m = _maxall(ls)
            es = [jnp.exp2((l - m) * (SCALE * LOG2E)) for l in ls]
            r = 1.0 / _addall(es)
            at = [e * r for e in es]
            for d0, d1 in zip(dv[:-1], dv[1:]):
                outs = []
                for d in range(d0, d1):
                    o = _addall([at[w] * kv[u - w + 8, pl.ds(D + d + DH * 8 * g, 8, stride=DH), :] for w in range(8)])
                    os_[pl.ds(d + DH * 8 * g, 8, stride=DH), :] = o
                    outs.append(o)
                last = _maxall(outs)
                if d1 < DH:
                    at = _after(last, at)

    def oproj_b(os_, ob):
        rhs = os_[pl.ds(0, D), :].astype(BF)
        MR = D // NO
        for i in range(NO):
            ob[pl.ds(64 + i * MR, MR), :] = jnp.dot(_unwords(wotb[pl.ds(i * MR // 2, MR // 2), :]), rhs,
                                                    preferred_element_type=F32)

    def otr_b(u, ob):
        wd = _words(ob[...].astype(BF).T)
        for cc in range(5):
            st[cc, pl.ds(u * PITCH, 64), :] = wd[:, 128 * cc:128 * cc + 128]

    qproj_b(0)
    attn(0, os0)
    p2(4)
    qproj_b(1)
    attn(1, os1)
    p2(6)
    oproj_b(os0, ob0)

    def p3(i, c):
        u = 2 * i
        ops = {'q': lambda k: qproj_b(u + k), 'a': lambda k: attn(u + k, (os0, os1)[k]),
               'o': lambda k: oproj_b((os1, os0)[k], (ob1, ob0)[k]), 't': lambda k: otr_b(u + k - 2, (ob0, ob1)[k])}
        for k in range(2):
            for ch in 'qaot':
                ops[ch](k)
        return c

    lax.fori_loop(1, NT // 2, p3, 0)
    oproj_b(os1, ob1)
    otr_b(NT - 2, ob0)
    otr_b(NT - 1, ob1)

    def qphi(t, os_):
        col = pl.ds(pl.multiple_of(t * 128, 128), 128)
        xt = xa_v[:, col]
        qs[pl.ds(0, D), :] = jnp.dot(_unwords(wta[pl.ds(0, D // 2), :]), xt, preferred_element_type=F32)
        for g in range(4):
            pq = [_phi(qs[pl.ds(d + DH * 8 * g, 8, stride=DH), :]) for d in range(DH)]
            den = _addall([pq[d] * zb[pl.ds(d + DH * 8 * g, 8, stride=DH), :] for d in range(DH)])
            r = 1.0 / (den + 1e-6)
            for d in range(DH):
                os_[pl.ds(d + DH * 8 * g, 8, stride=DH), :] = pq[d] * r

    def oproj_a(os_, ob):
        rhs = os_[pl.ds(0, D), :].astype(BF)
        ob[pl.ds(0, D), :] = jnp.dot(_unwords(mt[...]), rhs, preferred_element_type=F32)

    def emit(t, ob):
        oa = _words(ob[...].astype(BF).T)
        rws = pl.ds(pl.multiple_of(t * 128, 128), 128)
        outv[rws, pl.ds(0, 512)] = _unwords(oa[:, 0:512])
        for cc in range(5):
            wl = jnp.concatenate([st[cc, pl.ds(8 * half * PITCH + 4 * t + jj, 8, stride=PITCH), :]
                                  for jj in range(4) for half in range(2)], axis=0)
            if cc == 0:
                wl = wl | oa[:, 512:640]
            outv[rws, pl.ds(512 + 128 * cc, 128)] = _unwords(wl)

    def send(t):
        rws = pl.ds(pl.multiple_of(t * 128, 128), 128)
        pltpu.make_async_copy(outv.at[rws, :], out_h.at[rws, :], sem_out.at[0]).start()

    ob0[pl.ds(D, 64), :] = jnp.zeros((64, 128), F32)
    ob1[pl.ds(D, 64), :] = jnp.zeros((64, 128), F32)
    qphi(0, os0)
    qphi(1, os1)
    oproj_a(os0, ob0)

    def p4(i, c):
        t = 2 * i
        qphi(t, os0)
        oproj_a(os1, ob1)
        emit(t - 2, ob0)
        qphi(t + 1, os1)
        oproj_a(os0, ob0)
        emit(t - 1, ob1)
        send(t - 1)
        send(t - 2)
        return c

    p4(1, 0)
    lax.fori_loop(2, NT // 2, p4, 0)
    emit(NT - 2, ob0)
    send(NT - 2)
    oproj_a(os1, ob1)
    emit(NT - 1, ob1)
    send(NT - 1)
    pltpu.make_async_copy(outv, out_h, sem_out.at[0]).wait()


def make():
    any_spec = pl.BlockSpec(memory_space=pl.ANY)
    return pl.pallas_call(
        _kernel,
        out_shape=jax.ShapeDtypeStruct((S, 2 * D), BF),
        in_specs=[any_spec] * 6,
        out_specs=any_spec,
        scratch_shapes=[
            pltpu.VMEM((D, S), BF), pltpu.VMEM((D, 3 * D), BF), pltpu.VMEM((D, D), BF),
            pltpu.VMEM((D, S), BF), pltpu.VMEM((D, 3 * D), BF), pltpu.VMEM((D, D), BF),
            pltpu.VMEM((D, D), I32),
            pltpu.VMEM((3 * D // 2, D), I32),
            pltpu.VMEM((D // 2, D), I32),
            pltpu.VMEM((5, (NT + 1) * PITCH, 128), I32),
            pltpu.VMEM((24, D + RPAD, 128), F32),
            pltpu.VMEM((D // 2, S), I32),
            pltpu.VMEM((D // 2, D), I32),
            pltpu.VMEM((D, 128), F32),
            pltpu.VMEM((RPAD, 128), F32),
            pltpu.VMEM((D // 2, D), I32),
            pltpu.VMEM((RPAD, 128), F32),
            pltpu.VMEM((RPAD, 128), F32),
            pltpu.VMEM((RPAD, 128), F32),
            pltpu.VMEM((D + 64, 128), F32),
            pltpu.VMEM((D + 64, 128), F32),
            pltpu.VMEM((5, (NT + 1) * PITCH, 128), I32),
            pltpu.VMEM((S, 2 * D), BF),
            pltpu.SemaphoreType.DMA((12,)),
            pltpu.SemaphoreType.DMA((1,)),
        ],
        compiler_params=pltpu.CompilerParams(vmem_limit_bytes=100 * 1024 * 1024,
                                             flags={"XLA_TPU_RESCHEDULE_DMA_DONES": True}),
        name="fused_attn",
    )


@jax.jit
def pallas_concat_heads__linear_attn_block__sliding_local_dilated__prompt_kernel(A_x, A_wqkv, A_wo, B_x, B_wqkv, B_wo):
    out = make()(A_x[0].T, A_wqkv, A_wo, B_x[0].T, B_wqkv, B_wo)
    return out.reshape(1, S, 2 * D)
```

```python
import functools
import jax
import jax.numpy as jnp
from jax import lax
from jax.experimental import pallas as pl
from jax.experimental.pallas import tpu as pltpu

S = 2048
D = 576
DH = 18
NT = 16
RPAD = 600
PITCH = 68
BF = jnp.bfloat16
F32 = jnp.float32
I32 = jnp.int32
NT_DIMS = (((1,), (1,)), ((), ()))
BAND = ((0, 144), (112, 272), (240, 400), (368, 528), (496, 576))
SCALE = float(DH) ** -0.5
LOG2E = 1.4426950408889634


def _phi(t):
    return jnp.where(t > 0, t + 1.0, jnp.exp(t)) + 1e-6


def _words(x):
    return pltpu.bitcast(x, I32)


def _unwords(x):
    return pltpu.bitcast(x, BF)


def _addall(xs):
    return functools.reduce(lambda a, b: a + b, xs)


def _maxall(xs):
    return functools.reduce(jnp.maximum, xs)


def _after(tok, xs):
    never = jnp.abs(tok) < -1.0
    return [jnp.where(never, 0.0, x) for x in xs]


def _kernel(xa_h, wa_h, woa_h, xb_h, wb_h, wob_h, out_h,
            xa_v, wa_v, woa_v, xb_v, wb_v, wob_v,
            wta, wtb, wotb, xs, kv, pkt, pw, zacc, zb, mt, qs, os0, os1, ob0, ob1, st, outv,
            sem_in, sem_out):
    XC = 512
    cp_wak = pltpu.make_async_copy(wa_h.at[:, pl.ds(512, 640)], wa_v.at[:, pl.ds(512, 640)], sem_in.at[0])
    cp_xa = [pltpu.make_async_copy(xa_h.at[:, pl.ds(XC * i, XC)], xa_v.at[:, pl.ds(XC * i, XC)], sem_in.at[1 + i])
             for i in range(S // XC)]
    cp_wb = pltpu.make_async_copy(wb_h.at[:, pl.ds(512, 1216)], wb_v.at[:, pl.ds(512, 1216)], sem_in.at[5])
    cp_wbq = pltpu.make_async_copy(wb_h.at[:, pl.ds(0, 512)], wb_v.at[:, pl.ds(0, 512)], sem_in.at[11])
    cp_xb = pltpu.make_async_copy(xb_h, xb_v, sem_in.at[6])
    cp_wob = pltpu.make_async_copy(wob_h, wob_v, sem_in.at[7])
    cp_waq = pltpu.make_async_copy(wa_h.at[:, pl.ds(0, 512)], wa_v.at[:, pl.ds(0, 512)], sem_in.at[8])
    cp_wav = pltpu.make_async_copy(wa_h.at[:, pl.ds(1152, 576)], wa_v.at[:, pl.ds(1152, 576)], sem_in.at[9])
    cp_woa = pltpu.make_async_copy(woa_h, woa_v, sem_in.at[10])
    cp_wak.start()
    cp_xa[0].start()

    lane = lax.broadcasted_iota(I32, (8, 128), 1)

    cp_wak.wait()
    for c in cp_xa[1:]:
        c.start()
    cp_wb.start()
    cp_xb.start()
    cp_wob.start()
    cp_waq.start()
    cp_wav.start()
    cp_woa.start()
    cp_wbq.start()
    for c in range(4, 9):
        wta[pl.ds(64 * c, 64), :] = _words(wa_v[:, pl.ds(128 * c, 128)].T)
    zacc[...] = jnp.zeros((D, 128), F32)
    ob0[pl.ds(0, 64), :] = jnp.zeros((64, 128), F32)
    ob1[...] = jnp.zeros((D + 64, 128), F32)

    def p1(i, c):
        col = pl.ds(pl.multiple_of(i * XC, XC), XC)
        pltpu.make_async_copy(xa_h.at[:, col], xa_v.at[:, col], sem_in.at[1 + i]).wait()
        k = jnp.dot(_unwords(wta[pl.ds(D // 2, D // 2), :]), xa_v[:, col], preferred_element_type=F32)
        pk = _phi(k)
        pkt[:, col] = _words(pk.astype(BF))
        zacc[...] += _addall([pk[:, 128 * j:128 * j + 128] for j in range(XC // 128)])
        return c

    lax.fori_loop(0, S // XC, p1, 0)

    cp_wb.wait()
    cp_xb.wait()
    p = lax.dot_general(_unwords(pkt[...]), xa_v[...], NT_DIMS, preferred_element_type=F32)
    pw[...] = _words(p.astype(BF))
    zb[pl.ds(0, D), :] = jnp.broadcast_to(jnp.sum(zacc[...], axis=1, keepdims=True), (D, 128))
    for i in range(NT):
        wd = _words(xb_v[:, pl.ds(128 * i, 128)].T)
        for c in range(5):
            w = 128 if c < 4 else 64
            for r in range(8):
                start = 8 * (r % 2) * PITCH + 4 * i + r // 2
                xs[c, pl.ds(start, 8, stride=PITCH), pl.ds(0, w)] = wd[8 * r:8 * r + 8, 128 * c:128 * c + w]
    for c in range(4, 14):
        w = 128 if c < 13 else 64
        wtb[pl.ds(64 * c, w // 2), :] = _words(wb_v[:, pl.ds(128 * c, w)].T)

    cp_wob.wait()
    cp_waq.wait()
    cp_wav.wait()
    cp_woa.wait()
    cp_wbq.wait()
    for c in range(4):
        wtb[pl.ds(64 * c, 64), :] = _words(wb_v[:, pl.ds(128 * c, 128)].T)
    for c in range(5):
        w = 128 if c < 4 else 64
        wotb[pl.ds(64 * c, w // 2), :] = _words(wob_v[:, pl.ds(128 * c, w)].T)
    for c in range(4):
        wta[pl.ds(64 * c, 64), :] = _words(wa_v[:, pl.ds(128 * c, 128)].T)
    g_parts = []
    for jj in range(5):
        r0, r1 = BAND[jj]
        w = 128 if jj < 4 else 64
        g = jnp.dot(_unwords(pw[pl.ds(r0 // 2, (r1 - r0) // 2), :]), wa_v[:, pl.ds(2 * D + 128 * jj, w)],
                    preferred_element_type=F32)
        rr = lax.broadcasted_iota(I32, g.shape, 0) + r0
        cc = lax.broadcasted_iota(I32, g.shape, 1) + 128 * jj
        hr = lax.shift_right_logical(rr * 3641, 16)
        hc = lax.shift_right_logical(cc * 3641, 16)
        gb = jnp.where(hr == hc, g, 0.0).astype(BF)
        g_parts.append(gb)
    def load_xs(u):
        rws = pl.ds(u * PITCH, 64)
        parts = [xs[c, rws, :] for c in range(4)] + [xs[4, rws, pl.ds(0, 64)]]
        return _unwords(jnp.concatenate(parts, axis=1))

    def p2(u):
        xu = jnp.concatenate([load_xs(u), load_xs(u + 1)], axis=0)
        r = lax.dot_general(_unwords(wtb[pl.ds(D // 2, D), :]), xu, NT_DIMS, preferred_element_type=F32)
        for t in range(2):
            rt = r[:, 128 * t:128 * t + 128]
            kv[u + t + 8, pl.ds(0, 2 * D), :] = rt
            if u + t > 8:
                kv[u + t - 8, pl.ds(0, 2 * D), :] = pltpu.roll(rt, 2, 1)

    m_parts = [jnp.dot(g_parts[jj], woa_v[pl.ds(128 * jj, 128 if jj < 4 else 64), :], preferred_element_type=F32)
               for jj in range(5)]
    cuts = sorted(set([b for r in BAND for b in r]))
    rows = []
    for a, b in zip(cuts[:-1], cuts[1:]):
        rows.append(_addall([m_parts[jj][a - BAND[jj][0]:b - BAND[jj][0], :] for jj in range(5)
                             if BAND[jj][0] <= a and b <= BAND[jj][1]]))
    mt[...] = _words(jnp.concatenate(rows, axis=0).astype(BF).T)

    for u in (8, 10, 12, 14, 0, 2):
        p2(u)

    KL, KV, NM, NO = 4, 5, 3, 4
    MR = D // NM

    def qproj_b(u):
        xu = load_xs(u)
        for i in range(NM):
            qs[pl.ds(i * MR, MR), :] = lax.dot_general(_unwords(wtb[pl.ds(i * MR // 2, MR // 2), :]), xu, NT_DIMS,
                                                       preferred_element_type=F32)

    def attn(u, os_):
        last = None
        dk = [round(DH * i / KL) for i in range(KL + 1)]
        dv = [round(DH * i / KV) for i in range(KV + 1)]
        for g in range(4):
            q = [qs[pl.ds(d + DH * 8 * g, 8, stride=DH), :] for d in range(DH)]
            accs = [None] * 8
            for d0, d1 in zip(dk[:-1], dk[1:]):
                tok = last if d0 == 0 else _maxall(accs)
                qq = q[d0:d1]
                if tok is not None:
                    qq = _after(tok, qq)
                for w in range(8):
                    part = _addall([qq[d - d0] * kv[u - w + 8, pl.ds(d + DH * 8 * g, 8, stride=DH), :]
                                    for d in range(d0, d1)])
                    accs[w] = part if accs[w] is None else accs[w] + part
            ls = [accs[0]] + [jnp.where(lane >= jnp.where(u < w, 2, 0), accs[w], -1e9 / SCALE) for w in range(1, 8)]
            m = _maxall(ls)
            es = [jnp.exp2((l - m) * (SCALE * LOG2E)) for l in ls]
            r = 1.0 / _addall(es)
            at = [e * r for e in es]
            for d0, d1 in zip(dv[:-1], dv[1:]):
                outs = []
                for d in range(d0, d1):
                    o = _addall([at[w] * kv[u - w + 8, pl.ds(D + d + DH * 8 * g, 8, stride=DH), :] for w in range(8)])
                    os_[pl.ds(d + DH * 8 * g, 8, stride=DH), :] = o
                    outs.append(o)
                last = _maxall(outs)
                if d1 < DH:
                    at = _after(last, at)

    def oproj_b(os_, ob):
        rhs = os_[pl.ds(0, D), :].astype(BF)
        MR = D // NO
        for i in range(NO):
            ob[pl.ds(64 + i * MR, MR), :] = jnp.dot(_unwords(wotb[pl.ds(i * MR // 2, MR // 2), :]), rhs,
                                                    preferred_element_type=F32)

    def otr_b(u, ob):
        wd = _words(ob[...].astype(BF).T)
        for cc in range(5):
            st[cc, pl.ds(u * PITCH, 64), :] = wd[:, 128 * cc:128 * cc + 128]

    qproj_b(0)
    attn(0, os0)
    p2(4)
    qproj_b(1)
    attn(1, os1)
    p2(6)
    oproj_b(os0, ob0)

    def p3(i, c):
        for k, (os_cur, os_prev, ob_new, ob_old) in enumerate(((os0, os1, ob1, ob0), (os1, os0, ob0, ob1))):
            u = 2 * i + k
            qproj_b(u)
            attn(u, os_cur)
            oproj_b(os_prev, ob_new)
            otr_b(u - 2, ob_old)
        return c

    lax.fori_loop(1, NT // 2, p3, 0)
    oproj_b(os1, ob1)
    otr_b(NT - 2, ob0)
    otr_b(NT - 1, ob1)

    def qphi(t, os_):
        col = pl.ds(pl.multiple_of(t * 128, 128), 128)
        xt = xa_v[:, col]
        qs[pl.ds(0, D), :] = jnp.dot(_unwords(wta[pl.ds(0, D // 2), :]), xt, preferred_element_type=F32)
        for g in range(4):
            pq = [_phi(qs[pl.ds(d + DH * 8 * g, 8, stride=DH), :]) for d in range(DH)]
            den = _addall([pq[d] * zb[pl.ds(d + DH * 8 * g, 8, stride=DH), :] for d in range(DH)])
            r = 1.0 / (den + 1e-6)
            for d in range(DH):
                os_[pl.ds(d + DH * 8 * g, 8, stride=DH), :] = pq[d] * r

    def oproj_a(os_, ob):
        rhs = os_[pl.ds(0, D), :].astype(BF)
        ob[pl.ds(0, D), :] = jnp.dot(_unwords(mt[...]), rhs, preferred_element_type=F32)

    def emit(t, ob):
        oa = _words(ob[...].astype(BF).T)
        rws = pl.ds(pl.multiple_of(t * 128, 128), 128)
        outv[rws, pl.ds(0, 512)] = _unwords(oa[:, 0:512])
        for cc in range(5):
            wl = jnp.concatenate([st[cc, pl.ds(8 * half * PITCH + 4 * t + jj, 8, stride=PITCH), :]
                                  for jj in range(4) for half in range(2)], axis=0)
            if cc == 0:
                wl = wl | oa[:, 512:640]
            outv[rws, pl.ds(512 + 128 * cc, 128)] = _unwords(wl)

    def send(t):
        rws = pl.ds(pl.multiple_of(t * 128, 128), 128)
        pltpu.make_async_copy(outv.at[rws, :], out_h.at[rws, :], sem_out.at[0]).start()

    ob0[pl.ds(D, 64), :] = jnp.zeros((64, 128), F32)
    ob1[pl.ds(D, 64), :] = jnp.zeros((64, 128), F32)
    qphi(0, os0)
    qphi(1, os1)
    oproj_a(os0, ob0)

    def p4(i, c):
        t = 2 * i
        qphi(t, os0)
        oproj_a(os1, ob1)
        emit(t - 2, ob0)
        qphi(t + 1, os1)
        oproj_a(os0, ob0)
        emit(t - 1, ob1)
        send(t - 1)
        send(t - 2)
        return c

    p4(1, 0)
    lax.fori_loop(2, NT // 2, p4, 0)
    emit(NT - 2, ob0)
    send(NT - 2)
    oproj_a(os1, ob1)
    emit(NT - 1, ob1)
    send(NT - 1)
    pltpu.make_async_copy(outv, out_h, sem_out.at[0]).wait()


def make():
    any_spec = pl.BlockSpec(memory_space=pl.ANY)
    return pl.pallas_call(
        _kernel,
        out_shape=jax.ShapeDtypeStruct((S, 2 * D), BF),
        in_specs=[any_spec] * 6,
        out_specs=any_spec,
        scratch_shapes=[
            pltpu.VMEM((D, S), BF), pltpu.VMEM((D, 3 * D), BF), pltpu.VMEM((D, D), BF),
            pltpu.VMEM((D, S), BF), pltpu.VMEM((D, 3 * D), BF), pltpu.VMEM((D, D), BF),
            pltpu.VMEM((D, D), I32),
            pltpu.VMEM((3 * D // 2, D), I32),
            pltpu.VMEM((D // 2, D), I32),
            pltpu.VMEM((5, (NT + 1) * PITCH, 128), I32),
            pltpu.VMEM((24, D + RPAD, 128), F32),
            pltpu.VMEM((D // 2, S), I32),
            pltpu.VMEM((D // 2, D), I32),
            pltpu.VMEM((D, 128), F32),
            pltpu.VMEM((RPAD, 128), F32),
            pltpu.VMEM((D // 2, D), I32),
            pltpu.VMEM((RPAD, 128), F32),
            pltpu.VMEM((RPAD, 128), F32),
            pltpu.VMEM((RPAD, 128), F32),
            pltpu.VMEM((D + 64, 128), F32),
            pltpu.VMEM((D + 64, 128), F32),
            pltpu.VMEM((5, (NT + 1) * PITCH, 128), I32),
            pltpu.VMEM((S, 2 * D), BF),
            pltpu.SemaphoreType.DMA((12,)),
            pltpu.SemaphoreType.DMA((1,)),
        ],
        compiler_params=pltpu.CompilerParams(vmem_limit_bytes=100 * 1024 * 1024,
                                             flags={"XLA_TPU_RESCHEDULE_DMA_DONES": True}),
        name="fused_attn",
    )


@jax.jit
def pallas_concat_heads__linear_attn_block__sliding_local_dilated__prompt_kernel(A_x, A_wqkv, A_wo, B_x, B_wqkv, B_wo):
    out = make()(A_x[0].T, A_wqkv, A_wo, B_x[0].T, B_wqkv, B_wo)
    return out.reshape(1, S, 2 * D)
```
